```python
import os as _os
_os.environ.setdefault("JAX_PLATFORMS", "cpu")
import jax
import jax.numpy as jnp

def _softmax(x, axis=-1):
    return jax.nn.softmax(x, axis=axis)
def _gelu(x):
    return jax.nn.gelu(x, approximate=True)
def _silu(x):
    return jax.nn.silu(x)
def _sigmoid(x):
    return jax.nn.sigmoid(x)
def _layernorm(x, axis=-1, eps=1e-5):
    m = jnp.mean(x, axis=axis, keepdims=True)
    v = jnp.var(x, axis=axis, keepdims=True)
    return (x - m) / jnp.sqrt(v + eps)
def _scatter_add(tgt, idx, src, axis=0):
    return tgt.at[idx].add(src)
def _segment_sum(src, seg, n):
    return jax.ops.segment_sum(src, seg, n)
class _Rng:
    def __init__(self, key):
        self._k = key
    def _next(self):
        self._k, sub = jax.random.split(self._k)
        return sub
    def normal(self, shape):
        return jax.random.normal(self._next(), shape, dtype=jnp.bfloat16)
    def randint(self, lo, hi, shape):
        return jax.random.randint(self._next(), shape, lo, hi, dtype=jnp.int32)
    def uniform(self, shape, lo=0.0, hi=1.0):
        return jax.random.uniform(self._next(), shape, jnp.bfloat16, lo, hi)
    def permutation(self, n):
        return jax.random.permutation(self._next(), n)


kernel_name = 'concat_heads__mha_block_cached__mha_block_cached__near_ridge'

def setup_inputs():
    _rng = _Rng(jax.random.key(int.from_bytes(__import__("os").urandom(4), "little")))
    _w = (lambda a: (lambda t: t.astype(jnp.bfloat16) if jnp.issubdtype(t.dtype, jnp.floating) else t)(jnp.asarray(a)))
    def _A_setup():
        B, Sq, D = 8, 160, 512
        H, Sk, Dh = 32, 512, 128
        return {
            "x": _w((lambda *s: _rng.normal(s) * 0.8)(B, Sq, D)),
            "k_cache": _w((lambda *s: _rng.normal(s) * 0.8)(B, H, Sk, Dh)),
            "v_cache": _w((lambda *s: _rng.normal(s) * 0.05)(B, H, Sk, Dh)),
            "wq": _w((lambda *s: _rng.normal(s) * 0.8)(D, H * Dh) * (D ** -0.5)),
            "wo": _w((lambda *s: _rng.normal(s) * 0.05)(H * Dh, D) * ((H * Dh) ** -0.5)),
        }
    _A_in = _A_setup()

    def _B_setup():
        B, Sq, D = 8, 160, 512
        H, Sk, Dh = 32, 512, 128
        return {
            "x": _w((lambda *s: _rng.normal(s) * 0.8)(B, Sq, D)),
            "k_cache": _w((lambda *s: _rng.normal(s) * 0.8)(B, H, Sk, Dh)),
            "v_cache": _w((lambda *s: _rng.normal(s) * 0.05)(B, H, Sk, Dh)),
            "wq": _w((lambda *s: _rng.normal(s) * 0.8)(D, H * Dh) * (D ** -0.5)),
            "wo": _w((lambda *s: _rng.normal(s) * 0.05)(H * Dh, D) * ((H * Dh) ** -0.5)),
        }
    _B_in = _B_setup()

    return {
        "A_x": _A_in["x"],
        "A_k_cache": _A_in["k_cache"],
        "A_v_cache": _A_in["v_cache"],
        "A_wq": _A_in["wq"],
        "A_wo": _A_in["wo"],
        "B_x": _B_in["x"],
        "B_k_cache": _B_in["k_cache"],
        "B_v_cache": _B_in["v_cache"],
        "B_wq": _B_in["wq"],
        "B_wo": _B_in["wo"],
    }

def reference(A_x, A_k_cache, A_v_cache, A_wq, A_wo, B_x, B_k_cache, B_v_cache, B_wq, B_wo):
    def _A_ref(x, k_cache, v_cache, wq, wo):
        B, Sq, D = x.shape
        H, Dh = 32, 128
        q = (lambda x, *d: x.transpose(*d))((x @ wq).reshape(B, Sq, H, Dh), 0, 2, 1, 3)
        scores = jnp.einsum("bhqd,bhkd->bhqk", q, k_cache) * (Dh ** -0.5)
        p = _softmax(scores, axis=-1)
        o = jnp.einsum("bhqk,bhkd->bhqd", p, v_cache)
        return (lambda x, *d: x.transpose(*d))(o, 0, 2, 1, 3).reshape(B, Sq, H * Dh) @ wo

    def _B_ref(x, k_cache, v_cache, wq, wo):
        B, Sq, D = x.shape
        H, Dh = 32, 128
        q = (lambda x, *d: x.transpose(*d))((x @ wq).reshape(B, Sq, H, Dh), 0, 2, 1, 3)
        scores = jnp.einsum("bhqd,bhkd->bhqk", q, k_cache) * (Dh ** -0.5)
        p = _softmax(scores, axis=-1)
        o = jnp.einsum("bhqk,bhkd->bhqd", p, v_cache)
        return (lambda x, *d: x.transpose(*d))(o, 0, 2, 1, 3).reshape(B, Sq, H * Dh) @ wo

    a = _A_ref(A_x, A_k_cache, A_v_cache, A_wq, A_wo)
    b = _B_ref(B_x, B_k_cache, B_v_cache, B_wq, B_wo)
    return jnp.concatenate([a, b], axis=-1)
```

```python
import functools

import jax
import jax.numpy as jnp
from jax import lax
import jax.experimental.pallas as pl
import jax.experimental.pallas.tpu as pltpu

HB = 4


def _branch(x_ref, k_ref, v_ref, wq_ref, wo_ref, b, hb, dh, scale):
    x = x_ref[b]
    q = jnp.dot(x, wq_ref[...], preferred_element_type=jnp.float32)
    q = (q * scale).astype(jnp.bfloat16)
    outs = []
    for h in range(hb):
        qh = q[:, h * dh:(h + 1) * dh]
        s = lax.dot_general(qh, k_ref[0, h], (((1,), (1,)), ((), ())),
                            preferred_element_type=jnp.float32)
        m = jnp.max(s, axis=-1, keepdims=True)
        e = jnp.exp(s - m)
        l = jnp.sum(e, axis=-1, keepdims=True)
        o = jnp.dot(e.astype(jnp.bfloat16), v_ref[0, h],
                    preferred_element_type=jnp.float32)
        outs.append((o / l).astype(jnp.bfloat16))
    o = jnp.concatenate(outs, axis=-1)
    return jnp.dot(o, wo_ref[...], preferred_element_type=jnp.float32)


def _kernel(ax, ak, av, awq, awo, bx, bk, bv, bwq, bwo, out_ref, acc_ref, *, hb, dh, d, scale):
    hg = pl.program_id(0)
    b = pl.program_id(1)
    ya = _branch(ax, ak, av, awq, awo, b, hb, dh, scale)
    yb = _branch(bx, bk, bv, bwq, bwo, b, hb, dh, scale)
    y = jnp.concatenate([ya, yb], axis=-1)

    @pl.when(hg == 0)
    def _():
        acc_ref[b] = y

    @pl.when(hg > 0)
    def _():
        acc_ref[b] += y

    @pl.when(hg == pl.num_programs(0) - 1)
    def _():
        out_ref[b] = acc_ref[b].astype(out_ref.dtype)


@jax.jit
def pallas_concat_heads__mha_block_cached__mha_block_cached__near_ridge_kernel(
    A_x, A_k_cache, A_v_cache, A_wq, A_wo, B_x, B_k_cache, B_v_cache, B_wq, B_wo,
):
    B, Sq, D = A_x.shape
    _, H, Sk, Dh = A_k_cache.shape
    hb = HB
    scale = float(Dh) ** -0.5

    x_spec = pl.BlockSpec((B, Sq, D), lambda g, b: (0, 0, 0))
    kv_spec = pl.BlockSpec((1, hb, Sk, Dh), lambda g, b: (b, g, 0, 0))
    wq_spec = pl.BlockSpec((D, hb * Dh), lambda g, b: (0, g))
    wo_spec = pl.BlockSpec((hb * Dh, D), lambda g, b: (g, 0))
    in_specs = [x_spec, kv_spec, kv_spec, wq_spec, wo_spec] * 2
    out_spec = pl.BlockSpec((B, Sq, 2 * D), lambda g, b: (0, 0, 0))

    return pl.pallas_call(
        functools.partial(_kernel, hb=hb, dh=Dh, d=D, scale=scale),
        grid=(H // hb, B),
        in_specs=in_specs,
        out_specs=out_spec,
        out_shape=jax.ShapeDtypeStruct((B, Sq, 2 * D), jnp.bfloat16),
        scratch_shapes=[pltpu.VMEM((B, Sq, 2 * D), jnp.float32)],
        compiler_params=pltpu.CompilerParams(
            dimension_semantics=("arbitrary", "arbitrary"),
            vmem_limit_bytes=100 * 1024 * 1024,
        ),
    )(A_x, A_k_cache, A_v_cache, A_wq, A_wo, B_x, B_k_cache, B_v_cache, B_wq, B_wo)
```

```python
import functools
import jax
import jax.numpy as jnp
from jax import lax
import jax.experimental.pallas as pl
import jax.experimental.pallas.tpu as pltpu

LOG2E = 1.4426950408889634


def _kernel(ax, ak, av, awq, awo, bx, bk, bv, bwq, bwo, out_hbm,
            x_v, wq_v, wo_v, kv_v, acc_ref, ostage, x_sem, w_sem, kv_sem, o_sem,
            *, hb, dh, d, nb, ng, nslot, scale, depth):
    g = pl.program_id(0)
    b = pl.program_id(1)
    step = g * nb + b
    nsteps = ng * nb
    xs = (ax, bx)
    kvs = (ak, av, bk, bv)
    wqs = (awq, bwq)
    wos = (awo, bwo)
    cw = hb * dh

    def kv_copy(s, i):
        sg = s // nb
        sb = s % nb
        slot = s % nslot
        return pltpu.make_async_copy(
            kvs[i].at[sb, pl.ds(sg * hb, hb)], kv_v.at[slot, i], kv_sem.at[slot, i])

    def x_copy(j, bb):
        return pltpu.make_async_copy(xs[j].at[bb], x_v.at[j, bb], x_sem.at[j, bb])

    def wq_copy(j, gg):
        return pltpu.make_async_copy(
            wqs[j].at[:, pl.ds(gg * cw, cw)], wq_v.at[j, gg], w_sem.at[j])

    def wo_copy(j, gg):
        return pltpu.make_async_copy(
            wos[j].at[pl.ds(gg * cw, cw), :], wo_v.at[j, gg], w_sem.at[2 + j])

    def out_copy(bb):
        return pltpu.make_async_copy(ostage.at[bb], out_hbm.at[bb], o_sem.at[bb])

    @pl.when(step == 0)
    def _():
        for j in range(2):
            x_copy(j, 0).start()
            wq_copy(j, 0).start()
        for i in range(4):
            kv_copy(0, i).start()
        for j in range(2):
            wo_copy(j, 0).start()
        for s in range(1, nslot - 1):
            for i in range(4):
                kv_copy(s, i).start()
        for bb in range(1, nb):
            for j in range(2):
                x_copy(j, bb).start()

    nxt = step + nslot - 1

    @pl.when(nxt < nsteps)
    def _():
        for i in range(4):
            kv_copy(nxt, i).start()

    @pl.when(b == 0)
    def _():
        for j in range(2):
            wq_copy(j, g).wait()
            wo_copy(j, g).wait()

    @pl.when(jnp.logical_and(b == 0, g + 1 < ng))
    def _():
        for j in range(2):
            wq_copy(j, g + 1).start()
            wo_copy(j, g + 1).start()

    @pl.when(g == 0)
    def _():
        for j in range(2):
            x_copy(j, b).wait()
        acc_ref[b] = jnp.zeros(acc_ref.shape[1:], acc_ref.dtype)

    for i in range(4):
        kv_copy(step, i).wait()
    slot = step % nslot

    qs = []
    for j in range(2):
        q = jnp.dot(x_v[j, b], wq_v[j, g], preferred_element_type=jnp.float32)
        qs.append((q * (scale * LOG2E)).astype(jnp.bfloat16))

    tasks = [(j, h) for h in range(hb) for j in range(2)]

    def qk(t):
        j, h = t
        return lax.dot_general(qs[j][:, h * dh:(h + 1) * dh], kv_v[slot, 2 * j, h],
                               (((1,), (1,)), ((), ())), preferred_element_type=jnp.float32)

    ys = [None, None]

    def sm_pv(t, s):
        j, h = t
        m = jnp.max(s, axis=-1, keepdims=True)
        e = jnp.exp2(s - m)
        l = jnp.sum(e, axis=-1, keepdims=True)
        o = jnp.dot(e.astype(jnp.bfloat16), kv_v[slot, 2 * j + 1, h], preferred_element_type=jnp.float32)
        o = (o / l).astype(jnp.bfloat16)
        y = jnp.dot(o, wo_v[j, g, pl.ds(h * dh, dh), :], preferred_element_type=jnp.float32)
        ys[j] = y if ys[j] is None else ys[j] + y

    pend = []
    for t in tasks:
        pend.append((t, qk(t)))
        if len(pend) > depth:
            sm_pv(*pend.pop(0))
    while pend:
        sm_pv(*pend.pop(0))

    acc_ref[b] += jnp.concatenate(ys, axis=-1)

    @pl.when(g == ng - 1)
    def _():
        ostage[b] = acc_ref[b].astype(ostage.dtype)
        out_copy(b).start()

    @pl.when(step == nsteps - 1)
    def _():
        for bb in range(nb):
            out_copy(bb).wait()


HB = 4
NSLOT = 3
DEPTH = 1


@jax.jit
def pallas_concat_heads__mha_block_cached__mha_block_cached__near_ridge_kernel(
    A_x, A_k_cache, A_v_cache, A_wq, A_wo, B_x, B_k_cache, B_v_cache, B_wq, B_wo,
):
    hb, nslot, depth = HB, NSLOT, DEPTH
    B, Sq, D = A_x.shape
    _, H, Sk, Dh = A_k_cache.shape
    ng = H // hb
    scale = float(Dh) ** -0.5
    anyspec = pl.BlockSpec(memory_space=pl.ANY)
    return pl.pallas_call(
        functools.partial(_kernel, hb=hb, dh=Dh, d=D, nb=B, ng=ng, nslot=nslot, scale=scale, depth=depth),
        grid=(ng, B),
        in_specs=[anyspec] * 10,
        out_specs=anyspec,
        out_shape=jax.ShapeDtypeStruct((B, Sq, 2 * D), jnp.bfloat16),
        scratch_shapes=[
            pltpu.VMEM((2, B, Sq, D), jnp.bfloat16),
            pltpu.VMEM((2, ng, D, hb * Dh), jnp.bfloat16),
            pltpu.VMEM((2, ng, hb * Dh, D), jnp.bfloat16),
            pltpu.VMEM((nslot, 4, hb, Sk, Dh), jnp.bfloat16),
            pltpu.VMEM((B, Sq, 2 * D), jnp.float32),
            pltpu.VMEM((B, Sq, 2 * D), jnp.bfloat16),
            pltpu.SemaphoreType.DMA((2, B)),
            pltpu.SemaphoreType.DMA((4,)),
            pltpu.SemaphoreType.DMA((nslot, 4)),
            pltpu.SemaphoreType.DMA((B,)),
        ],
        compiler_params=pltpu.CompilerParams(
            dimension_semantics=("arbitrary", "arbitrary"),
            vmem_limit_bytes=110 * 1024 * 1024,
        ),
    )(A_x, A_k_cache, A_v_cache, A_wq, A_wo, B_x, B_k_cache, B_v_cache, B_wq, B_wo)
```

```python
import functools
import jax
import jax.numpy as jnp
from jax import lax
import jax.experimental.pallas as pl
import jax.experimental.pallas.tpu as pltpu

LOG2E = 1.4426950408889634


def _kernel(ax, ak, av, awq, awo, bx, bk, bv, bwq, bwo, out_hbm,
            x_v, wq_v, wo_v, kv_v, q_v, acc_ref, ostage, x_sem, wq_sem, wo_sem, kv_sem, o_sem,
            *, hb, dh, d, nb, ng, nslot, scale, ipos, wb, sq):
    g = pl.program_id(0)
    b = pl.program_id(1)
    step = g * nb + b
    nsteps = ng * nb
    xs = (ax, bx)
    kvs = (ak, av, bk, bv)
    wqs = (awq, bwq)
    wos = (awo, bwo)
    cw = hb * dh

    def kv_copy(s, i):
        sg = s // nb
        sb = s % nb
        slot = s % nslot
        return pltpu.make_async_copy(
            kvs[i].at[sb, pl.ds(sg * hb, hb)], kv_v.at[slot, i], kv_sem.at[slot, i])

    def x_copy(j):
        return pltpu.make_async_copy(xs[j], x_v.at[j], x_sem.at[j])

    def wq_copy(j, gg):
        return pltpu.make_async_copy(
            wqs[j].at[:, pl.ds(gg * cw, cw)], wq_v.at[j, gg % 2], wq_sem.at[j])

    def wo_copy(j, gg):
        return pltpu.make_async_copy(
            wos[j].at[pl.ds(gg * cw, cw), :], wo_v.at[j, gg % 2], wo_sem.at[j])

    def out_copy(bb):
        return pltpu.make_async_copy(ostage.at[bb], out_hbm.at[bb], o_sem.at[bb])

    def qlump(j, r0=0, r1=None):
        r1 = nb if r1 is None else r1
        xa = x_v[j, r0:r1].reshape((r1 - r0) * sq, d)
        q = jnp.dot(xa, wq_v[j, g % 2], preferred_element_type=jnp.float32)
        q_v[j, r0 * sq:r1 * sq, :] = (q * (scale * LOG2E)).astype(jnp.bfloat16)

    @pl.when(step == 0)
    def _():
        hbn = nb // 2
        x_copy(0).start()
        wq_copy(0, 0).start()
        x_copy(0).wait()
        x_copy(1).start()
        wq_copy(1, 0).start()
        wq_copy(0, 0).wait()
        qlump(0, 0, hbn)
        x_copy(1).wait()
        for i in range(4):
            kv_copy(0, i).start()
        wq_copy(1, 0).wait()
        qlump(0, hbn, nb)
        kv_copy(0, 0).wait()
        for j in range(2):
            wo_copy(j, 0).start()
        kv_copy(0, 1).wait()
        qlump(1, 0, hbn)
        kv_copy(0, 2).wait()
        for s in range(1, nslot - 1):
            for i in range(4):
                kv_copy(s, i).start()
        kv_copy(0, 3).wait()
        qlump(1, hbn, nb)
        for j in range(2):
            wo_copy(j, 0).wait()

    @pl.when(jnp.logical_and(b == 0, g > 0))
    def _():
        for j in range(2):
            wq_copy(j, g).wait()
        for j in range(2):
            qlump(j)
        for j in range(2):
            wo_copy(j, g).wait()

    @pl.when(g == 0)
    def _():
        acc_ref[b] = jnp.zeros(acc_ref.shape[1:], acc_ref.dtype)

    @pl.when(step > 0)
    def _():
        for i in range(4):
            kv_copy(step, i).wait()
    slot = step % nslot
    row0 = pl.multiple_of(b * sq, 16)

    def issue_prefetch():
        nxt = step + nslot - 1

        @pl.when(nxt < nsteps)
        def _():
            for i in range(4):
                kv_copy(nxt, i).start()

        @pl.when(jnp.logical_and(b == wb, g + 1 < ng))
        def _():
            for j in range(2):
                wq_copy(j, g + 1).start()
                wo_copy(j, g + 1).start()

    tasks = [(j, h) for h in range(hb) for j in range(2)]

    def qk(t):
        j, h = t
        return lax.dot_general(q_v[j, pl.ds(row0, sq), pl.ds(h * dh, dh)], kv_v[slot, 2 * j, h],
                               (((1,), (1,)), ((), ())), preferred_element_type=jnp.float32)

    def sm_pv(t, s):
        j, h = t
        m = jnp.max(s, axis=-1, keepdims=True)
        e = jnp.exp2(s - m)
        l = jnp.sum(e, axis=-1, keepdims=True)
        o = jnp.dot(e.astype(jnp.bfloat16), kv_v[slot, 2 * j + 1, h], preferred_element_type=jnp.float32)
        o = (o / l).astype(jnp.bfloat16)
        y = jnp.dot(o, wo_v[j, g % 2, pl.ds(h * dh, dh), :], preferred_element_type=jnp.float32)
        acc_ref[b, :, j * d:(j + 1) * d] += y

    pend = []
    for idx, t in enumerate(tasks):
        pend.append((t, qk(t)))
        if idx == ipos:
            issue_prefetch()
        if len(pend) > 1:
            sm_pv(*pend.pop(0))
    while pend:
        sm_pv(*pend.pop(0))

    @pl.when(g == ng - 1)
    def _():
        ostage[b] = acc_ref[b].astype(ostage.dtype)
        out_copy(b).start()

    @pl.when(step == nsteps - 1)
    def _():
        for bb in range(nb):
            out_copy(bb).wait()


HB = 8
NSLOT = 4
WB = 1


@jax.jit
def pallas_concat_heads__mha_block_cached__mha_block_cached__near_ridge_kernel(
    A_x, A_k_cache, A_v_cache, A_wq, A_wo, B_x, B_k_cache, B_v_cache, B_wq, B_wo,
):
    hb, nslot, wb = HB, NSLOT, WB
    B, Sq, D = A_x.shape
    _, H, Sk, Dh = A_k_cache.shape
    ng = H // hb
    scale = float(Dh) ** -0.5
    anyspec = pl.BlockSpec(memory_space=pl.ANY)
    return pl.pallas_call(
        functools.partial(_kernel, hb=hb, dh=Dh, d=D, nb=B, ng=ng, nslot=nslot, scale=scale, ipos=0,
                          wb=wb, sq=Sq),
        grid=(ng, B),
        in_specs=[anyspec] * 10,
        out_specs=anyspec,
        out_shape=jax.ShapeDtypeStruct((B, Sq, 2 * D), jnp.bfloat16),
        scratch_shapes=[
            pltpu.VMEM((2, B, Sq, D), jnp.bfloat16),
            pltpu.VMEM((2, 2, D, hb * Dh), jnp.bfloat16),
            pltpu.VMEM((2, 2, hb * Dh, D), jnp.bfloat16),
            pltpu.VMEM((nslot, 4, hb, Sk, Dh), jnp.bfloat16),
            pltpu.VMEM((2, B * Sq, hb * Dh), jnp.bfloat16),
            pltpu.VMEM((B, Sq, 2 * D), jnp.float32),
            pltpu.VMEM((B, Sq, 2 * D), jnp.bfloat16),
            pltpu.SemaphoreType.DMA((2,)),
            pltpu.SemaphoreType.DMA((2,)),
            pltpu.SemaphoreType.DMA((2,)),
            pltpu.SemaphoreType.DMA((nslot, 4)),
            pltpu.SemaphoreType.DMA((B,)),
        ],
        compiler_params=pltpu.CompilerParams(
            dimension_semantics=("arbitrary", "arbitrary"),
            vmem_limit_bytes=120 * 1024 * 1024,
        ),
    )(A_x, A_k_cache, A_v_cache, A_wq, A_wo, B_x, B_k_cache, B_v_cache, B_wq, B_wo)
```

```python
import functools
import jax
import jax.numpy as jnp
from jax import lax
import jax.experimental.pallas as pl
import jax.experimental.pallas.tpu as pltpu

LOG2E = 1.4426950408889634


def _kernel(ax, ak, av, awq, awo, bx, bk, bv, bwq, bwo, out_hbm,
            x_v, wq_v, wo_v, kv_v, q_v, acc_ref, ostage, x_sem, wq_sem, wo_sem, kv_sem, o_sem,
            *, hb, dh, d, nb, ng, nslot, scale, wb, sq, P):
    g = pl.program_id(0)
    bb = pl.program_id(1)
    nbb = nb // P
    step = g * nbb + bb
    nsteps = ng * nbb
    xs = (ax, bx)
    kvs = (ak, av, bk, bv)
    wqs = (awq, bwq)
    wos = (awo, bwo)
    cw = hb * dh

    def kv_copy(s, p, i):
        sg = s // nbb
        sb = (s % nbb) * P + p
        slot = s % nslot
        return pltpu.make_async_copy(
            kvs[i].at[sb, pl.ds(sg * hb, hb)], kv_v.at[slot, p, i], kv_sem.at[slot, p, i])

    def x_copy(j):
        return pltpu.make_async_copy(xs[j], x_v.at[j], x_sem.at[j])

    def wq_copy(j, gg):
        return pltpu.make_async_copy(
            wqs[j].at[:, pl.ds(gg * cw, cw)], wq_v.at[j, gg % 2], wq_sem.at[j])

    def wo_copy(j, gg):
        return pltpu.make_async_copy(
            wos[j].at[pl.ds(gg * cw, cw), :], wo_v.at[j, gg % 2], wo_sem.at[j])

    def out_copy(b_):
        return pltpu.make_async_copy(ostage.at[b_], out_hbm.at[b_], o_sem.at[b_])

    def qlump(j, par, r0=0, r1=None):
        r1 = nb if r1 is None else r1
        xa = x_v[j, r0:r1].reshape((r1 - r0) * sq, d)
        q = jnp.dot(xa, wq_v[j, par], preferred_element_type=jnp.float32)
        q_v[par, j, r0 * sq:r1 * sq, :] = (q * (scale * LOG2E)).astype(jnp.bfloat16)

    kv_ids = [(p, i) for p in range(P) for i in range(4)]

    @pl.when(step == 0)
    def _():
        hbn = nb // 2
        x_copy(0).start()
        wq_copy(0, 0).start()
        x_copy(0).wait()
        x_copy(1).start()
        wq_copy(1, 0).start()
        wq_copy(0, 0).wait()
        qlump(0, 0, 0, hbn)
        x_copy(1).wait()
        wq_copy(0, 1).start()
        wq_copy(1, 0).wait()
        wq_copy(1, 1).start()
        qlump(0, 0, hbn, nb)
        wq_copy(0, 1).wait()
        for p, i in kv_ids[:4]:
            kv_copy(0, p, i).start()
        wq_copy(1, 1).wait()
        qlump(1, 0, 0, hbn)
        kv_copy(0, 0, 0).wait()
        for j in range(2):
            wo_copy(j, 0).start()
        for p, i in kv_ids[4:]:
            kv_copy(0, p, i).start()
        kv_copy(0, 0, 1).wait()
        qlump(1, 0, hbn, nb)
        kv_copy(0, 0, 2).wait()
        for p, i in kv_ids:
            kv_copy(1, p, i).start()
        kv_copy(0, 0, 3).wait()
        qlump(0, 1)
        for j in range(2):
            wo_copy(j, 0).wait()
        for s in range(2, nslot - 1):
            for p, i in kv_ids:
                kv_copy(s, p, i).start()
        kv_copy(0, 1, 0).wait()
        qlump(1, 1)
        for p, i in kv_ids[5:]:
            kv_copy(0, p, i).wait()

    @pl.when(jnp.logical_and(bb == 0, g > 0))
    def _():
        for j in range(2):
            wo_copy(j, g).wait()

        @pl.when(g + 1 < ng)
        def _():
            for j in range(2):
                wq_copy(j, g + 1).wait()
            for j in range(2):
                qlump(j, (g + 1) % 2)

    @pl.when(g == 0)
    def _():
        acc_ref[pl.ds(bb * P, P)] = jnp.zeros((P,) + acc_ref.shape[1:], acc_ref.dtype)

    @pl.when(step > 0)
    def _():
        for p, i in kv_ids:
            kv_copy(step, p, i).wait()

    slot = step % nslot

    def issue_prefetch():
        nxt = step + nslot - 1

        @pl.when(nxt < nsteps)
        def _():
            for p, i in kv_ids:
                kv_copy(nxt, p, i).start()

        @pl.when(jnp.logical_and(bb == wb, g + 1 < ng))
        def _():
            for j in range(2):
                wo_copy(j, g + 1).start()

        @pl.when(jnp.logical_and(bb == wb, g + 2 < ng))
        def _():
            for j in range(2):
                wq_copy(j, g + 2).start()

    tasks = [(p, j, h) for p in range(P) for h in range(hb) for j in range(2)]

    def qk(t):
        p, j, h = t
        row0 = pl.multiple_of((bb * P + p) * sq, 16)
        return lax.dot_general(q_v[g % 2, j, pl.ds(row0, sq), pl.ds(h * dh, dh)], kv_v[slot, p, 2 * j, h],
                               (((1,), (1,)), ((), ())), preferred_element_type=jnp.float32)

    def sm_pv(t, s):
        p, j, h = t
        m = jnp.max(s, axis=-1, keepdims=True)
        e = jnp.exp2(s - m)
        l = jnp.sum(e, axis=-1, keepdims=True)
        o = jnp.dot(e.astype(jnp.bfloat16), kv_v[slot, p, 2 * j + 1, h], preferred_element_type=jnp.float32)
        o = (o / l).astype(jnp.bfloat16)
        y = jnp.dot(o, wo_v[j, g % 2, pl.ds(h * dh, dh), :], preferred_element_type=jnp.float32)
        acc_ref[bb * P + p, :, j * d:(j + 1) * d] += y

    pend = []
    for idx, t in enumerate(tasks):
        pend.append((t, qk(t)))
        if idx == 0:
            issue_prefetch()
        if len(pend) > 1:
            sm_pv(*pend.pop(0))
    while pend:
        sm_pv(*pend.pop(0))

    @pl.when(g == ng - 1)
    def _():
        for p in range(P):
            b_ = bb * P + p
            ostage[b_] = acc_ref[b_].astype(ostage.dtype)
            out_copy(b_).start()

    @pl.when(step == nsteps - 1)
    def _():
        for b_ in range(nb):
            out_copy(b_).wait()


HB = 8
NSLOT = 4
WB = 0
PB = 2


@jax.jit
def pallas_concat_heads__mha_block_cached__mha_block_cached__near_ridge_kernel(
    A_x, A_k_cache, A_v_cache, A_wq, A_wo, B_x, B_k_cache, B_v_cache, B_wq, B_wo,
):
    hb, nslot, wb, P = HB, NSLOT, WB, PB
    B, Sq, D = A_x.shape
    _, H, Sk, Dh = A_k_cache.shape
    ng = H // hb
    scale = float(Dh) ** -0.5
    anyspec = pl.BlockSpec(memory_space=pl.ANY)
    return pl.pallas_call(
        functools.partial(_kernel, hb=hb, dh=Dh, d=D, nb=B, ng=ng, nslot=nslot, scale=scale,
                          wb=wb, sq=Sq, P=P),
        grid=(ng, B // P),
        in_specs=[anyspec] * 10,
        out_specs=anyspec,
        out_shape=jax.ShapeDtypeStruct((B, Sq, 2 * D), jnp.bfloat16),
        scratch_shapes=[
            pltpu.VMEM((2, B, Sq, D), jnp.bfloat16),
            pltpu.VMEM((2, 2, D, hb * Dh), jnp.bfloat16),
            pltpu.VMEM((2, 2, hb * Dh, D), jnp.bfloat16),
            pltpu.VMEM((nslot, P, 4, hb, Sk, Dh), jnp.bfloat16),
            pltpu.VMEM((2, 2, B * Sq, hb * Dh), jnp.bfloat16),
            pltpu.VMEM((B, Sq, 2 * D), jnp.float32),
            pltpu.VMEM((B, Sq, 2 * D), jnp.bfloat16),
            pltpu.SemaphoreType.DMA((2,)),
            pltpu.SemaphoreType.DMA((2,)),
            pltpu.SemaphoreType.DMA((2,)),
            pltpu.SemaphoreType.DMA((nslot, P, 4)),
            pltpu.SemaphoreType.DMA((B,)),
        ],
        compiler_params=pltpu.CompilerParams(
            dimension_semantics=("arbitrary", "arbitrary"),
            vmem_limit_bytes=120 * 1024 * 1024,
        ),
    )(A_x, A_k_cache, A_v_cache, A_wq, A_wo, B_x, B_k_cache, B_v_cache, B_wq, B_wo)
```

```python
import functools
import jax
import jax.numpy as jnp
from jax import lax
import jax.experimental.pallas as pl
import jax.experimental.pallas.tpu as pltpu

LOG2E = 1.4426950408889634


def _kernel(ax, ak, av, awq, awo, bx, bk, bv, bwq, bwo, out_hbm,
            x_v, wq_v, wo_v, kv_v, q_v, acc_ref, ostage, x_sem, wq_sem, wo_sem, kv_sem, o_sem,
            *, hb, dh, d, nb, ng, nslot, scale, wb, sq, P):
    g = pl.program_id(0)
    bb = pl.program_id(1)
    nbb = nb // P
    step = g * nbb + bb
    nsteps = ng * nbb
    xs = (ax, bx)
    kvs = (ak, av, bk, bv)
    wqs = (awq, bwq)
    wos = (awo, bwo)
    cw = hb * dh

    def kv_copy(s, p, i):
        sg = s // nbb
        sb = (s % nbb) * P + p
        slot = s % nslot
        return pltpu.make_async_copy(
            kvs[i].at[sb, pl.ds(sg * hb, hb)], kv_v.at[slot, p, i], kv_sem.at[slot, p, i])

    def x_copy(j, hf):
        hn = nb // 2
        return pltpu.make_async_copy(xs[j].at[pl.ds(hf * hn, hn)], x_v.at[j, pl.ds(hf * hn, hn)], x_sem.at[j, hf])

    def wq_copy(j, gg):
        return pltpu.make_async_copy(
            wqs[j].at[:, pl.ds(gg * cw, cw)], wq_v.at[j, gg % 2], wq_sem.at[j])

    def wo_copy(j, gg):
        return pltpu.make_async_copy(
            wos[j].at[pl.ds(gg * cw, cw), :], wo_v.at[j, gg % 2], wo_sem.at[j])

    def out_copy(b_):
        return pltpu.make_async_copy(ostage.at[b_], out_hbm.at[b_], o_sem.at[b_])

    def qlump(j, par, r0=0, r1=None):
        r1 = nb if r1 is None else r1
        xa = x_v[j, r0:r1].reshape((r1 - r0) * sq, d)
        q = jnp.dot(xa, wq_v[j, par], preferred_element_type=jnp.float32)
        q_v[par, j, r0 * sq:r1 * sq, :] = (q * (scale * LOG2E)).astype(jnp.bfloat16)

    kv_ids = [(p, i) for p in range(P) for i in range(4)]

    @pl.when(step == 0)
    def _():
        hbn = nb // 2
        x_copy(0, 0).start()
        wq_copy(0, 0).start()
        acc_ref[...] = jnp.zeros(acc_ref.shape, acc_ref.dtype)
        x_copy(0, 0).wait()
        x_copy(0, 1).start()
        x_copy(1, 0).start()
        x_copy(1, 1).start()
        wq_copy(1, 0).start()
        wq_copy(0, 0).wait()
        qlump(0, 0, 0, hbn)
        x_copy(0, 1).wait()
        x_copy(1, 0).wait()
        x_copy(1, 1).wait()
        wq_copy(0, 1).start()
        wq_copy(1, 0).wait()
        wq_copy(1, 1).start()
        qlump(0, 0, hbn, nb)
        wq_copy(0, 1).wait()
        for p, i in kv_ids[:4]:
            kv_copy(0, p, i).start()
        wq_copy(1, 1).wait()
        qlump(1, 0, 0, hbn)
        kv_copy(0, 0, 0).wait()
        for j in range(2):
            wo_copy(j, 0).start()
        for p, i in kv_ids[4:]:
            kv_copy(0, p, i).start()
        kv_copy(0, 0, 1).wait()
        qlump(1, 0, hbn, nb)
        kv_copy(0, 0, 2).wait()
        for p, i in kv_ids:
            kv_copy(1, p, i).start()
        kv_copy(0, 0, 3).wait()
        qlump(0, 1)
        for j in range(2):
            wo_copy(j, 0).wait()
        for s in range(2, nslot - 1):
            for p, i in kv_ids:
                kv_copy(s, p, i).start()
        kv_copy(0, 1, 0).wait()
        qlump(1, 1)
        for p, i in kv_ids[5:]:
            kv_copy(0, p, i).wait()

    @pl.when(jnp.logical_and(bb == 0, g > 0))
    def _():
        for j in range(2):
            wo_copy(j, g).wait()

        @pl.when(g + 1 < ng)
        def _():
            for j in range(2):
                wq_copy(j, g + 1).wait()
            for j in range(2):
                qlump(j, (g + 1) % 2)

    @pl.when(step > 0)
    def _():
        for p, i in kv_ids:
            kv_copy(step, p, i).wait()

    slot = step % nslot

    def issue_prefetch():
        nxt = step + nslot - 1

        @pl.when(nxt < nsteps)
        def _():
            for p, i in kv_ids:
                kv_copy(nxt, p, i).start()

        @pl.when(jnp.logical_and(bb == wb, g + 1 < ng))
        def _():
            for j in range(2):
                wo_copy(j, g + 1).start()

        @pl.when(jnp.logical_and(bb == wb, g + 2 < ng))
        def _():
            for j in range(2):
                wq_copy(j, g + 2).start()

    tasks = [(p, j, h) for p in range(P) for h in range(hb) for j in range(2)]

    def qk(t):
        p, j, h = t
        row0 = pl.multiple_of((bb * P + p) * sq, 16)
        return lax.dot_general(q_v[g % 2, j, pl.ds(row0, sq), pl.ds(h * dh, dh)], kv_v[slot, p, 2 * j, h],
                               (((1,), (1,)), ((), ())), preferred_element_type=jnp.float32)

    def sm_pv(t, s):
        p, j, h = t
        m = jnp.max(s, axis=-1, keepdims=True)
        e = jnp.exp2(s - m)
        l = jnp.sum(e, axis=-1, keepdims=True)
        o = jnp.dot(e.astype(jnp.bfloat16), kv_v[slot, p, 2 * j + 1, h], preferred_element_type=jnp.float32)
        o = (o / l).astype(jnp.bfloat16)
        y = jnp.dot(o, wo_v[j, g % 2, pl.ds(h * dh, dh), :], preferred_element_type=jnp.float32)
        acc_ref[bb * P + p, :, j * d:(j + 1) * d] += y

    pend = []
    for idx, t in enumerate(tasks):
        pend.append((t, qk(t)))
        if idx == 0:
            issue_prefetch()
        if len(pend) > 1:
            sm_pv(*pend.pop(0))
    while pend:
        sm_pv(*pend.pop(0))

    @pl.when(g == ng - 1)
    def _():
        for p in range(P):
            b_ = bb * P + p
            ostage[b_] = acc_ref[b_].astype(ostage.dtype)
            out_copy(b_).start()

    @pl.when(step == nsteps - 1)
    def _():
        for b_ in range(nb):
            out_copy(b_).wait()


HB = 8
NSLOT = 4
WB = 0
PB = 2


@jax.jit
def pallas_concat_heads__mha_block_cached__mha_block_cached__near_ridge_kernel(
    A_x, A_k_cache, A_v_cache, A_wq, A_wo, B_x, B_k_cache, B_v_cache, B_wq, B_wo,
):
    hb, nslot, wb, P = HB, NSLOT, WB, PB
    B, Sq, D = A_x.shape
    _, H, Sk, Dh = A_k_cache.shape
    ng = H // hb
    scale = float(Dh) ** -0.5
    anyspec = pl.BlockSpec(memory_space=pl.ANY)
    return pl.pallas_call(
        functools.partial(_kernel, hb=hb, dh=Dh, d=D, nb=B, ng=ng, nslot=nslot, scale=scale,
                          wb=wb, sq=Sq, P=P),
        grid=(ng, B // P),
        in_specs=[anyspec] * 10,
        out_specs=anyspec,
        out_shape=jax.ShapeDtypeStruct((B, Sq, 2 * D), jnp.bfloat16),
        scratch_shapes=[
            pltpu.VMEM((2, B, Sq, D), jnp.bfloat16),
            pltpu.VMEM((2, 2, D, hb * Dh), jnp.bfloat16),
            pltpu.VMEM((2, 2, hb * Dh, D), jnp.bfloat16),
            pltpu.VMEM((nslot, P, 4, hb, Sk, Dh), jnp.bfloat16),
            pltpu.VMEM((2, 2, B * Sq, hb * Dh), jnp.bfloat16),
            pltpu.VMEM((B, Sq, 2 * D), jnp.float32),
            pltpu.VMEM((B, Sq, 2 * D), jnp.bfloat16),
            pltpu.SemaphoreType.DMA((2, 2)),
            pltpu.SemaphoreType.DMA((2,)),
            pltpu.SemaphoreType.DMA((2,)),
            pltpu.SemaphoreType.DMA((nslot, P, 4)),
            pltpu.SemaphoreType.DMA((B,)),
        ],
        compiler_params=pltpu.CompilerParams(
            dimension_semantics=("arbitrary", "arbitrary"),
            vmem_limit_bytes=120 * 1024 * 1024,
        ),
    )(A_x, A_k_cache, A_v_cache, A_wq, A_wo, B_x, B_k_cache, B_v_cache, B_wq, B_wo)
```

```python
import functools

import jax
import jax.numpy as jnp
from jax import lax
import jax.experimental.pallas as pl
import jax.experimental.pallas.tpu as pltpu

LOG2E = 1.4426950408889634


def _kernel(ax, ak, av, awq, awo, bx, bk, bv, bwq, bwo, out_hbm,
            x_v, wq_v, wo_v, kv_v, q_v, acc_ref, ostage, x_sem, wq_sem, wo_sem, kv_sem, o_sem,
            *, hb, dh, d, nb, ng, nslot, scale, wb, sq, P):
    g = pl.program_id(0)
    bb = pl.program_id(1)
    nbb = nb // P
    step = g * nbb + bb
    nsteps = ng * nbb
    xs = (ax, bx)
    kvs = (ak, av, bk, bv)
    wqs = (awq, bwq)
    wos = (awo, bwo)
    cw = hb * dh

    def kv_copy(s, p, i):
        sg = s // nbb
        sb = (s % nbb) * P + p
        slot = s % nslot
        return pltpu.make_async_copy(
            kvs[i].at[sb, pl.ds(sg * hb, hb)], kv_v.at[slot, p, i], kv_sem.at[slot, p, i])

    def x_copy(j, hf):
        hn = nb // 2
        return pltpu.make_async_copy(
            xs[j].at[pl.ds(hf * hn, hn)], x_v.at[j, pl.ds(hf * hn, hn)], x_sem.at[j, hf])

    def wq_copy(j, gg):
        return pltpu.make_async_copy(
            wqs[j].at[:, pl.ds(gg * cw, cw)], wq_v.at[j, gg % 2], wq_sem.at[j])

    def wo_copy(j, gg):
        return pltpu.make_async_copy(
            wos[j].at[pl.ds(gg * cw, cw), :], wo_v.at[j, gg % 2], wo_sem.at[j])

    def out_copy(b_):
        return pltpu.make_async_copy(ostage.at[b_], out_hbm.at[b_], o_sem.at[b_])

    def qlump(j, par, r0=0, r1=None):
        r1 = nb if r1 is None else r1
        xa = x_v[j, r0:r1].reshape((r1 - r0) * sq, d)
        q = jnp.dot(xa, wq_v[j, par], preferred_element_type=jnp.float32)
        q_v[par, j, r0 * sq:r1 * sq, :] = q.astype(jnp.bfloat16)

    kv_ids = [(p, i) for p in range(P) for i in range(4)]

    @pl.when(step == 0)
    def _():
        hbn = nb // 2
        x_copy(0, 0).start()
        wq_copy(0, 0).start()
        acc_ref[...] = jnp.zeros(acc_ref.shape, acc_ref.dtype)
        x_copy(0, 0).wait()
        x_copy(0, 1).start()
        x_copy(1, 0).start()
        x_copy(1, 1).start()
        wq_copy(1, 0).start()
        wq_copy(0, 0).wait()
        qlump(0, 0, 0, hbn)
        x_copy(0, 1).wait()
        x_copy(1, 0).wait()
        x_copy(1, 1).wait()
        wq_copy(0, 1).start()
        wq_copy(1, 0).wait()
        wq_copy(1, 1).start()
        qlump(0, 0, hbn, nb)
        wq_copy(0, 1).wait()
        for p, i in kv_ids[:4]:
            kv_copy(0, p, i).start()
        wq_copy(1, 1).wait()
        qlump(1, 0, 0, hbn)
        kv_copy(0, 0, 0).wait()
        for j in range(2):
            wo_copy(j, 0).start()
        for p, i in kv_ids[4:]:
            kv_copy(0, p, i).start()
        kv_copy(0, 0, 1).wait()
        qlump(1, 0, hbn, nb)
        kv_copy(0, 0, 2).wait()
        for p, i in kv_ids:
            kv_copy(1, p, i).start()
        kv_copy(0, 0, 3).wait()
        qlump(0, 1)
        for j in range(2):
            wo_copy(j, 0).wait()
        for s in range(2, nslot - 1):
            for p, i in kv_ids:
                kv_copy(s, p, i).start()
        kv_copy(0, 1, 0).wait()
        qlump(1, 1)
        for p, i in kv_ids[5:]:
            kv_copy(0, p, i).wait()

    @pl.when(jnp.logical_and(bb == 0, g > 0))
    def _():
        for j in range(2):
            wo_copy(j, g).wait()

        @pl.when(g + 1 < ng)
        def _():
            for j in range(2):
                wq_copy(j, g + 1).wait()
            for j in range(2):
                qlump(j, (g + 1) % 2)

    @pl.when(step > 0)
    def _():
        for p, i in kv_ids:
            kv_copy(step, p, i).wait()

    slot = step % nslot

    def issue_prefetch():
        nxt = step + nslot - 1

        @pl.when(nxt < nsteps)
        def _():
            for p, i in kv_ids:
                kv_copy(nxt, p, i).start()

        @pl.when(jnp.logical_and(bb == wb, g + 1 < ng))
        def _():
            for j in range(2):
                wo_copy(j, g + 1).start()

        @pl.when(jnp.logical_and(bb == wb, g + 2 < ng))
        def _():
            for j in range(2):
                wq_copy(j, g + 2).start()

    tasks = [(p, j, h) for p in range(P) for h in range(hb) for j in range(2)]

    def qk(t):
        p, j, h = t
        row0 = pl.multiple_of((bb * P + p) * sq, 16)
        return lax.dot_general(q_v[g % 2, j, pl.ds(row0, sq), pl.ds(h * dh, dh)], kv_v[slot, p, 2 * j, h],
                               (((1,), (1,)), ((), ())), preferred_element_type=jnp.float32)

    def sm_pv(t, s):
        p, j, h = t
        m = jnp.max(s, axis=-1, keepdims=True)
        e = jnp.exp2((s - m) * (scale * LOG2E))
        l = jnp.sum(e, axis=-1, keepdims=True)
        o = jnp.dot(e.astype(jnp.bfloat16), kv_v[slot, p, 2 * j + 1, h], preferred_element_type=jnp.float32)
        o = (o / l).astype(jnp.bfloat16)
        y = jnp.dot(o, wo_v[j, g % 2, pl.ds(h * dh, dh), :], preferred_element_type=jnp.float32)
        acc_ref[bb * P + p, :, j * d:(j + 1) * d] += y

    pend = []
    for idx, t in enumerate(tasks):
        pend.append((t, qk(t)))
        if idx == 0:
            issue_prefetch()
        if len(pend) > 1:
            sm_pv(*pend.pop(0))
    while pend:
        sm_pv(*pend.pop(0))

    @pl.when(g == ng - 1)
    def _():
        for p in range(P):
            b_ = bb * P + p
            ostage[b_] = acc_ref[b_].astype(ostage.dtype)
            out_copy(b_).start()

    @pl.when(step == nsteps - 1)
    def _():
        for b_ in range(nb):
            out_copy(b_).wait()


HB = 8
NSLOT = 4
WB = 0
PB = 2


@jax.jit
def pallas_concat_heads__mha_block_cached__mha_block_cached__near_ridge_kernel(
    A_x, A_k_cache, A_v_cache, A_wq, A_wo, B_x, B_k_cache, B_v_cache, B_wq, B_wo,
):
    hb, nslot, wb, P = HB, NSLOT, WB, PB
    B, Sq, D = A_x.shape
    _, H, Sk, Dh = A_k_cache.shape
    ng = H // hb
    assert H % hb == 0 and ng >= 2 and B % P == 0 and B % 2 == 0 and Sq % 16 == 0
    assert ng * (B // P) >= nslot
    scale = float(Dh) ** -0.5
    anyspec = pl.BlockSpec(memory_space=pl.ANY)
    return pl.pallas_call(
        functools.partial(_kernel, hb=hb, dh=Dh, d=D, nb=B, ng=ng, nslot=nslot, scale=scale,
                          wb=wb, sq=Sq, P=P),
        grid=(ng, B // P),
        in_specs=[anyspec] * 10,
        out_specs=anyspec,
        out_shape=jax.ShapeDtypeStruct((B, Sq, 2 * D), jnp.bfloat16),
        scratch_shapes=[
            pltpu.VMEM((2, B, Sq, D), jnp.bfloat16),
            pltpu.VMEM((2, 2, D, hb * Dh), jnp.bfloat16),
            pltpu.VMEM((2, 2, hb * Dh, D), jnp.bfloat16),
            pltpu.VMEM((nslot, P, 4, hb, Sk, Dh), jnp.bfloat16),
            pltpu.VMEM((2, 2, B * Sq, hb * Dh), jnp.bfloat16),
            pltpu.VMEM((B, Sq, 2 * D), jnp.float32),
            pltpu.VMEM((B, Sq, 2 * D), jnp.bfloat16),
            pltpu.SemaphoreType.DMA((2, 2)),
            pltpu.SemaphoreType.DMA((2,)),
            pltpu.SemaphoreType.DMA((2,)),
            pltpu.SemaphoreType.DMA((nslot, P, 4)),
            pltpu.SemaphoreType.DMA((B,)),
        ],
        compiler_params=pltpu.CompilerParams(
            dimension_semantics=("arbitrary", "arbitrary"),
            vmem_limit_bytes=120 * 1024 * 1024,
        ),
    )(A_x, A_k_cache, A_v_cache, A_wq, A_wo, B_x, B_k_cache, B_v_cache, B_wq, B_wo)
```
